```python
import os as _os
_os.environ.setdefault("JAX_PLATFORMS", "cpu")
import jax
import jax.numpy as jnp

def _softmax(x, axis=-1):
    return jax.nn.softmax(x, axis=axis)
def _gelu(x):
    return jax.nn.gelu(x, approximate=True)
def _silu(x):
    return jax.nn.silu(x)
def _sigmoid(x):
    return jax.nn.sigmoid(x)
def _layernorm(x, axis=-1, eps=1e-5):
    m = jnp.mean(x, axis=axis, keepdims=True)
    v = jnp.var(x, axis=axis, keepdims=True)
    return (x - m) / jnp.sqrt(v + eps)
def _scatter_add(tgt, idx, src, axis=0):
    return tgt.at[idx].add(src)
def _segment_sum(src, seg, n):
    return jax.ops.segment_sum(src, seg, n)
class _Rng:
    def __init__(self, key):
        self._k = key
    def _next(self):
        self._k, sub = jax.random.split(self._k)
        return sub
    def normal(self, shape):
        return jax.random.normal(self._next(), shape, dtype=jnp.bfloat16)
    def randint(self, lo, hi, shape):
        return jax.random.randint(self._next(), shape, lo, hi, dtype=jnp.int32)
    def uniform(self, shape, lo=0.0, hi=1.0):
        return jax.random.uniform(self._next(), shape, jnp.bfloat16, lo, hi)
    def permutation(self, n):
        return jax.random.permutation(self._next(), n)


kernel_name = 'sequential_preLN__softmax_full_mha__glu_gated_swiglu__prompt'

def setup_inputs():
    _rng = _Rng(jax.random.key(int.from_bytes(__import__("os").urandom(4), "little")))
    _w = (lambda a: (lambda t: t.astype(jnp.bfloat16) if jnp.issubdtype(t.dtype, jnp.floating) else t)(jnp.asarray(a)))
    def _A_setup():
        B, S, D = 1, 2048, 640
        return {
            "x": _w((lambda *s: _rng.normal(s) * 0.05)(B, S, D)),
            "wqkv": _w((lambda *s: _rng.normal(s) * 0.05)(D, 3 * D)),
            "wo": _w((lambda *s: _rng.normal(s) * 0.05)(D, D)),
        }
    _A_in = _A_setup()

    def _B_setup():
        B, S, D, F = 1, 2048, 640, 1728
        return {
            "x": _w((lambda *s: _rng.normal(s) * 0.05)(B, S, D)),
            "w1": _w((lambda *s: _rng.normal(s) * 0.05)(D, F) * (2.0 / D) ** 0.5),
            "w3": _w((lambda *s: _rng.normal(s) * 0.05)(D, F) * (2.0 / D) ** 0.5),
            "w2": _w((lambda *s: _rng.normal(s) * 0.05)(F, D) * (2.0 / F) ** 0.5),
        }
    _B_in = _B_setup()

    return {
        "A_x": _A_in["x"],
        "A_wqkv": _A_in["wqkv"],
        "A_wo": _A_in["wo"],
        "B_x": _B_in["x"],
        "B_w1": _B_in["w1"],
        "B_w3": _B_in["w3"],
        "B_w2": _B_in["w2"],
    }

def reference(A_x, A_wqkv, A_wo, B_x, B_w1, B_w3, B_w2):
    def _A_ref(x, wqkv, wo):
        B, S, D = x.shape
        H = 32; Dh = D // H
        qkv = (lambda x, *d: x.transpose(*d))((x @ wqkv).reshape(B, S, 3, H, Dh), 2, 0, 3, 1, 4)
        q, k, v = qkv[0], qkv[1], qkv[2]
        scale = Dh ** -0.5
        scores = jnp.einsum("bhqd,bhkd->bhqk", q, k) * scale
        p = _softmax(scores, axis=-1)
        o = jnp.einsum("bhqk,bhkd->bhqd", p, v)
        return (lambda x, *d: x.transpose(*d))(o, 0, 2, 1, 3).reshape(B, S, D) @ wo

    def _B_ref(x, w1, w3, w2):
        gate = jnp.einsum("bsd,df->bsf", x, w1)
        up = jnp.einsum("bsd,df->bsf", x, w3)
        h = _silu(gate) * up
        out = jnp.einsum("bsf,fd->bsd", h, w2)
        return out

    x = A_x
    h = x + _A_ref(_layernorm(x, axis=-1), A_wqkv, A_wo)
    h2 = h + _B_ref(_layernorm(h, axis=-1), B_w1, B_w3, B_w2)
    return h2
```

```python
import functools
import jax
import jax.numpy as jnp
import jax.experimental.pallas as pl
import jax.experimental.pallas.tpu as pltpu

S = 2048
D = 640
H = 32
DH = 20
F = 1728
EPS = 1e-5
LOG2E = 1.4426950408889634
HPS = 6
NSLAB = 6
QKW = NSLAB * 128
HR = 24
TQ = 512
CK = 128
TR = 256


def _ln(x):
    m = jnp.mean(x, axis=-1, keepdims=True)
    xc = x - m
    v = jnp.mean(xc * xc, axis=-1, keepdims=True)
    return xc * jax.lax.rsqrt(v + EPS)


def kernel(x_ref, wqkv_ref, wo_ref, w1_ref, w3_ref, w2_ref, out_ref,
           wp_s, wo_s, q_s, k_s, vt_s, o_s, s_a, s_b, m_a, m_b):
    nq = S // TQ
    N = H * nq
    nc = S // CK

    wp_s[...] = jnp.zeros_like(wp_s)
    wq_all = wqkv_ref[...]
    for t in range(2):
        for h in range(H):
            lo = 128 * (h // HPS) + DH * (h % HPS)
            wp_s[:, t * QKW + lo: t * QKW + lo + DH] = wq_all[:, t * D + h * DH: t * D + (h + 1) * DH]
    wp_s[:, 2 * QKW: 2 * QKW + D] = wq_all[:, 2 * D: 3 * D]
    wo_s[...] = jnp.zeros_like(wo_s)
    wo_all = wo_ref[...].astype(jnp.float32)
    for h in range(H):
        wo_s[h * HR: h * HR + DH, :] = wo_all[h * DH: (h + 1) * DH, :]
    vt_s[...] = jnp.zeros_like(vt_s)
    vt_s[:, DH:DH + 1, :] = jnp.ones((H, 1, S), jnp.bfloat16)

    def p0(r, c):
        rows = pl.ds(pl.multiple_of(r * TR, TR), TR)
        xn = _ln(x_ref[rows, :].astype(jnp.float32)).astype(jnp.bfloat16)
        qkv = jnp.dot(xn, wp_s[...], preferred_element_type=jnp.float32)
        q_s[rows, :] = (qkv[:, 0:QKW] * (DH ** -0.5 * LOG2E)).astype(jnp.bfloat16)
        k_s[rows, :] = qkv[:, QKW:2 * QKW].astype(jnp.bfloat16)
        vT = qkv[:, 2 * QKW:2 * QKW + D].T
        for h in range(H):
            vt_s[h, 0:DH, rows] = vT[h * DH:(h + 1) * DH, :].astype(jnp.bfloat16)
        return c
    jax.lax.fori_loop(0, S // TR, p0, 0)

    lane = jax.lax.broadcasted_iota(jnp.int32, (TQ, 128), 1)
    rowi = jax.lax.broadcasted_iota(jnp.int32, (HR, TQ), 0)

    def step(jn, j, s_next, m_next, s_cur, m_cur, first=False):
        hn = jn // nq
        jqn = jn % nq
        h = j // nq
        jq = j % nq
        sl = hn // HPS
        lo = DH * (hn % HPS)
        slab = pl.ds(pl.multiple_of(sl * 128, 128), 128)
        qn = q_s[pl.ds(pl.multiple_of(jqn * TQ, TQ), TQ), slab]
        qn = jnp.where((lane >= lo) & (lane < lo + DH), qn, jnp.zeros_like(qn))
        if not first:
            m = m_cur[...]
        acc = None
        mrun = None
        for c in range(nc):
            ks = pl.ds(c * CK, CK)
            sT = jax.lax.dot_general(k_s[ks, slab], qn, (((1,), (1,)), ((), ())),
                                     preferred_element_type=jnp.float32)
            s_next[ks, :] = sT
            mc = jnp.max(sT, axis=0, keepdims=True)
            mrun = mc if mrun is None else jnp.maximum(mrun, mc)
            if not first:
                pT = jnp.exp2(s_cur[ks, :] - m).astype(jnp.bfloat16)
                d = jnp.dot(vt_s[h, :, ks], pT, preferred_element_type=jnp.float32)
                acc = d if acc is None else acc + d
        m_next[...] = mrun
        if not first:
            inv = 1.0 / acc[DH:DH + 1, :]
            o = jnp.where(rowi < DH, acc[0:HR, :] * inv, 0.0)
            o_s[h, :, pl.ds(pl.multiple_of(jq * TQ, TQ), TQ)] = o

    step(0, 0, s_a, m_a, None, None, first=True)

    def body(i, c):
        j = 2 * i
        step(j + 1, j, s_b, m_b, s_a, m_a)
        step(jnp.minimum(j + 2, N - 1), j + 1, s_a, m_a, s_b, m_b)
        return c
    jax.lax.fori_loop(0, N // 2, body, 0)

    def p2(r, c):
        rows = pl.ds(pl.multiple_of(r * TR, TR), TR)
        oT = o_s[:, :, rows].reshape(H * HR, TR).astype(jnp.bfloat16)
        attn = jax.lax.dot_general(oT, wo_s[...].astype(jnp.bfloat16), (((0,), (0,)), ((), ())),
                                   preferred_element_type=jnp.float32)
        hres = x_ref[rows, :].astype(jnp.float32) + attn
        hn = _ln(hres).astype(jnp.bfloat16)
        g = jnp.dot(hn, w1_ref[...], preferred_element_type=jnp.float32)
        u = jnp.dot(hn, w3_ref[...], preferred_element_type=jnp.float32)
        a = (g * (1.0 / (1.0 + jnp.exp(-g))) * u).astype(jnp.bfloat16)
        y = jnp.dot(a, w2_ref[...], preferred_element_type=jnp.float32)
        out_ref[rows, :] = (hres + y).astype(out_ref.dtype)
        return c
    jax.lax.fori_loop(0, S // TR, p2, 0)


@jax.jit
def pallas_sequential_preLN__softmax_full_mha__glu_gated_swiglu__prompt_kernel(A_x, A_wqkv, A_wo, B_x, B_w1, B_w3, B_w2):
    x = A_x.reshape(S, D)
    out = pl.pallas_call(
        kernel,
        out_shape=jax.ShapeDtypeStruct((S, D), A_x.dtype),
        scratch_shapes=[
            pltpu.VMEM((D, 2 * QKW + D), jnp.bfloat16),
            pltpu.VMEM((H * HR, D), jnp.float32),
            pltpu.VMEM((S, QKW), jnp.bfloat16),
            pltpu.VMEM((S, QKW), jnp.bfloat16),
            pltpu.VMEM((H, 32, S), jnp.bfloat16),
            pltpu.VMEM((H, HR, S), jnp.float32),
            pltpu.VMEM((S, TQ), jnp.float32),
            pltpu.VMEM((S, TQ), jnp.float32),
            pltpu.VMEM((1, TQ), jnp.float32),
            pltpu.VMEM((1, TQ), jnp.float32),
        ],
        compiler_params=pltpu.CompilerParams(vmem_limit_bytes=110 * 1024 * 1024),
    )(x, A_wqkv, A_wo, B_w1, B_w3, B_w2)
    return out.reshape(A_x.shape)
```

```python
import jax
import jax.numpy as jnp
import jax.experimental.pallas as pl
import jax.experimental.pallas.tpu as pltpu

S = 2048
D = 640
H = 32
DH = 20
F = 1728
EPS = 1e-5
LOG2E = 1.4426950408889634
HPS = 6
NSLAB = 6
QKW = NSLAB * 128
HR = 24
TQ = 512
CK = 128
TR = 512


def _ln(x):
    m = jnp.mean(x, axis=-1, keepdims=True)
    xc = x - m
    v = jnp.mean(xc * xc, axis=-1, keepdims=True)
    return xc * jax.lax.rsqrt(v + EPS)


def kernel(x_hbm, wqkv_ref, wo_hbm, w1_hbm, w3_hbm, w2_hbm, out_hbm,
           x_ref, wo_ref, w1_ref, w3_ref, w2_ref, sems, out_buf, osems, wp_s, wvt_s, wo_s, q_s, k_s, vt_s, o_s, s_a, s_b, m_a, m_b):
    nq = S // TQ
    N = H * nq
    nc = S // CK

    x_copy = pltpu.make_async_copy(x_hbm, x_ref, sems.at[4])
    x_copy.start()
    copies = [pltpu.make_async_copy(src, dst, sems.at[i])
              for i, (src, dst) in enumerate(((wo_hbm, wo_ref), (w1_hbm, w1_ref),
                                              (w3_hbm, w3_ref), (w2_hbm, w2_ref)))]
    for cp in copies:
        cp.start()
    wp_s[...] = jnp.zeros_like(wp_s)
    wq_all = wqkv_ref[...]
    for t in range(2):
        for h in range(H):
            lo = 128 * (h // HPS) + DH * (h % HPS)
            wp_s[:, t * QKW + lo: t * QKW + lo + DH] = wq_all[:, t * D + h * DH: t * D + (h + 1) * DH]
    wvt_s[...] = wq_all[:, 2 * D: 3 * D].astype(jnp.float32).T.astype(jnp.bfloat16)
    vt_s[:, DH:, :] = jnp.where(jax.lax.broadcasted_iota(jnp.int32, (H, 32 - DH, S), 1) == 0,
                                1.0, 0.0).astype(jnp.bfloat16)

    x_copy.wait()
    def p0(r, c):
        rows = pl.ds(pl.multiple_of(r * TR, TR), TR)
        xn = _ln(x_ref[rows, :].astype(jnp.float32)).astype(jnp.bfloat16)
        qkv = jnp.dot(xn, wp_s[...], preferred_element_type=jnp.float32)
        q_s[rows, :] = (qkv[:, 0:QKW] * (DH ** -0.5 * LOG2E)).astype(jnp.bfloat16)
        k_s[rows, :] = qkv[:, QKW:2 * QKW].astype(jnp.bfloat16)
        vT = jax.lax.dot_general(wvt_s[...], xn, (((1,), (1,)), ((), ())),
                                 preferred_element_type=jnp.float32)
        for h in range(H):
            vt_s[h, 0:DH, rows] = vT[h * DH:(h + 1) * DH, :].astype(jnp.bfloat16)
        return c
    jax.lax.fori_loop(0, S // TR, p0, 0)

    lane = jax.lax.broadcasted_iota(jnp.int32, (TQ, 128), 1)
    rowi = jax.lax.broadcasted_iota(jnp.int32, (HR, TQ), 0)

    def step(jn, j, s_next, m_next, s_cur, m_cur, first=False):
        hn = jn // nq
        jqn = jn % nq
        h = j // nq
        jq = j % nq
        sl = hn // HPS
        lo = DH * (hn % HPS)
        slab = pl.ds(pl.multiple_of(sl * 128, 128), 128)
        qn = q_s[pl.ds(pl.multiple_of(jqn * TQ, TQ), TQ), slab]
        qn = jnp.where((lane >= lo) & (lane < lo + DH), qn, jnp.zeros_like(qn))
        if not first:
            m = m_cur[...]
        acc = None
        mrun = None
        for c in range(nc):
            ks = pl.ds(c * CK, CK)
            sT = jax.lax.dot_general(k_s[ks, slab], qn, (((1,), (1,)), ((), ())),
                                     preferred_element_type=jnp.float32)
            s_next[ks, :] = sT
            mc = jnp.max(sT, axis=0, keepdims=True)
            mrun = mc if mrun is None else jnp.maximum(mrun, mc)
            if not first:
                pT = jnp.exp2(s_cur[ks, :] - m).astype(jnp.bfloat16)
                d = jnp.dot(vt_s[h, :, ks], pT, preferred_element_type=jnp.float32)
                acc = d if acc is None else acc + d
        m_next[...] = mrun
        if not first:
            inv = 1.0 / acc[DH:DH + 1, :]
            o = jnp.where(rowi < DH, acc[0:HR, :] * inv, 0.0)
            o_s[h, :, pl.ds(pl.multiple_of(jq * TQ, TQ), TQ)] = o

    step(0, 0, s_a, m_a, None, None, first=True)

    def body(i, c):
        j = 2 * i
        step(j + 1, j, s_b, m_b, s_a, m_a)
        step(jnp.minimum(j + 2, N - 1), j + 1, s_a, m_a, s_b, m_b)
        return c
    jax.lax.fori_loop(0, N // 2, body, 0)

    for cp in copies:
        cp.wait()
    wo_s[...] = jnp.zeros_like(wo_s)
    wo_all = wo_ref[...].astype(jnp.float32)
    for h in range(H):
        wo_s[h * HR: h * HR + DH, :] = wo_all[h * DH: (h + 1) * DH, :]
    def p2(r, c):
        rows = pl.ds(pl.multiple_of(r * TR, TR), TR)
        oT = o_s[:, :, rows].reshape(H * HR, TR).astype(jnp.bfloat16)
        attn = jax.lax.dot_general(oT, wo_s[...].astype(jnp.bfloat16), (((0,), (0,)), ((), ())),
                                   preferred_element_type=jnp.float32)
        hres = x_ref[rows, :].astype(jnp.float32) + attn
        hn = _ln(hres).astype(jnp.bfloat16)
        g = jax.lax.dot_general(hn, w1_ref[...], (((1,), (1,)), ((), ())), preferred_element_type=jnp.float32)
        u = jax.lax.dot_general(hn, w3_ref[...], (((1,), (1,)), ((), ())), preferred_element_type=jnp.float32)
        a = (g * (1.0 / (1.0 + jnp.exp(-g))) * u).astype(jnp.bfloat16)
        y = jnp.dot(a, w2_ref[...], preferred_element_type=jnp.float32)
        slot = r % 2

        @pl.when(r >= 2)
        def _():
            out_copy(r - 2, slot).wait()
        out_buf[slot] = (hres + y).astype(out_buf.dtype)
        out_copy(r, slot).start()
        return c

    def out_copy(r, slot):
        return pltpu.make_async_copy(out_buf.at[slot], out_hbm.at[pl.ds(pl.multiple_of(r * TR, TR), TR), :],
                                     osems.at[slot])
    nr = S // TR
    jax.lax.fori_loop(0, nr, p2, 0)
    out_copy(nr - 2, (nr - 2) % 2).wait()
    out_copy(nr - 1, (nr - 1) % 2).wait()


@jax.jit
def pallas_sequential_preLN__softmax_full_mha__glu_gated_swiglu__prompt_kernel(A_x, A_wqkv, A_wo, B_x, B_w1, B_w3, B_w2):
    x = A_x.reshape(S, D)
    out = pl.pallas_call(
        kernel,
        out_shape=jax.ShapeDtypeStruct((S, D), A_x.dtype),
        out_specs=pl.BlockSpec(memory_space=pl.ANY),
        in_specs=[pl.BlockSpec(memory_space=pl.ANY), pl.BlockSpec(memory_space=pltpu.VMEM)]
        + [pl.BlockSpec(memory_space=pl.ANY)] * 4,
        scratch_shapes=[
            pltpu.VMEM((S, D), jnp.bfloat16),
            pltpu.VMEM((D, D), jnp.bfloat16), pltpu.VMEM((F, D), jnp.bfloat16),
            pltpu.VMEM((F, D), jnp.bfloat16), pltpu.VMEM((F, D), jnp.bfloat16),
            pltpu.SemaphoreType.DMA((5,)),
            pltpu.VMEM((2, TR, D), jnp.bfloat16), pltpu.SemaphoreType.DMA((2,)),
            pltpu.VMEM((D, 2 * QKW), jnp.bfloat16),
            pltpu.VMEM((D, D), jnp.bfloat16),
            pltpu.VMEM((H * HR, D), jnp.float32),
            pltpu.VMEM((S, QKW), jnp.bfloat16),
            pltpu.VMEM((S, QKW), jnp.bfloat16),
            pltpu.VMEM((H, 32, S), jnp.bfloat16),
            pltpu.VMEM((H, HR, S), jnp.float32),
            pltpu.VMEM((S, TQ), jnp.float32),
            pltpu.VMEM((S, TQ), jnp.float32),
            pltpu.VMEM((1, TQ), jnp.float32),
            pltpu.VMEM((1, TQ), jnp.float32),
        ],
        compiler_params=pltpu.CompilerParams(vmem_limit_bytes=110 * 1024 * 1024),
    )(x, A_wqkv, A_wo, B_w1.T, B_w3.T, B_w2)
    return out.reshape(A_x.shape)
```
